```python
import os as _os
_os.environ.setdefault("JAX_PLATFORMS", "cpu")
import jax
import jax.numpy as jnp

def _softmax(x, axis=-1):
    return jax.nn.softmax(x, axis=axis)
def _gelu(x):
    return jax.nn.gelu(x, approximate=True)
def _silu(x):
    return jax.nn.silu(x)
def _sigmoid(x):
    return jax.nn.sigmoid(x)
def _layernorm(x, axis=-1, eps=1e-5):
    m = jnp.mean(x, axis=axis, keepdims=True)
    v = jnp.var(x, axis=axis, keepdims=True)
    return (x - m) / jnp.sqrt(v + eps)
def _scatter_add(tgt, idx, src, axis=0):
    return tgt.at[idx].add(src)
def _segment_sum(src, seg, n):
    return jax.ops.segment_sum(src, seg, n)
class _Rng:
    def __init__(self, key):
        self._k = key
    def _next(self):
        self._k, sub = jax.random.split(self._k)
        return sub
    def normal(self, shape):
        return jax.random.normal(self._next(), shape, dtype=jnp.bfloat16)
    def randint(self, lo, hi, shape):
        return jax.random.randint(self._next(), shape, lo, hi, dtype=jnp.int32)
    def uniform(self, shape, lo=0.0, hi=1.0):
        return jax.random.uniform(self._next(), shape, jnp.bfloat16, lo, hi)
    def permutation(self, n):
        return jax.random.permutation(self._next(), n)


kernel_name = 'standalone__seq2seq_rnn_t_joint__speech'

def setup_inputs():
    _rng = _Rng(jax.random.key(int.from_bytes(__import__("os").urandom(4), "little")))
    _w = (lambda a: (lambda t: t.astype(jnp.bfloat16) if jnp.issubdtype(t.dtype, jnp.floating) else t)(jnp.asarray(a)))
    B, T, D, K = 2, 1000, 512, 31
    U = 8
    sc = (1.0 / (K * D)) ** 0.5
    sd = (1.0 / D) ** 0.5
    return {
        "x": _w((lambda *s: _rng.normal(s) * 0.4)(B, T, D) * 0.5),
        "w1": _w((lambda *s: _rng.normal(s) * 1.6)(K, D, D) * sc),
        "w2": _w((lambda *s: _rng.normal(s) * 1.6)(K, D, D) * sc),
        "g": _w((lambda *s: _rng.normal(s) * 1.6)(B, U, D) * 0.5),
        "w_f": _w((lambda *s: _rng.normal(s) * 1.6)(D, D) * sd),
        "w_g": _w((lambda *s: _rng.normal(s) * 1.6)(D, D) * sd),
        "w_o": _w((lambda *s: _rng.normal(s) * 1.6)(D, D) * sd),
    }

def reference(x, w1, w2, g, w_f, w_g, w_o):
    B, T, D = x.shape
    K = w1.shape[0]
    pad = K // 2
    xp = jnp.pad(x, ((0,0),(pad,pad),(0,0)))
    h = jnp.zeros_like(x)
    for i in range(K):
        h = h + jnp.einsum("btc,cd->btd", xp[:, i:i+T, :], w1[i])
    h = _gelu(h)[:, ::2, :]
    T1 = h.shape[1]
    hp = jnp.pad(h, ((0,0),(pad,pad),(0,0)))
    f = jnp.zeros_like(h)
    for i in range(K):
        f = f + jnp.einsum("btc,cd->btd", hp[:, i:i+T1, :], w2[i])
    f = _gelu(f)[:, ::2, :]
    fe = jnp.einsum("btd,de->bte", f, w_f)
    ge = jnp.einsum("bud,de->bue", g, w_g)
    j = jnp.tanh(fe[:, :, None, :] + ge[:, None, :, :])
    return jnp.einsum("btud,dv->btuv", j, w_o)
```

```python
import jax
import jax.numpy as jnp
import jax.experimental.pallas as pl
import jax.experimental.pallas.tpu as pltpu

F32 = jnp.float32
BF16 = jnp.bfloat16
U32 = jnp.uint32

B, T, D, KT, NU = 2, 1000, 512, 31, 8
NL = 128
NCH = D // NL
M = 64
XP_ROWS = 1096
HB_BLK = 80
HB_ROWS = 16 * HB_BLK + 16
W_SRC = 0
W_ST = 256
W_L2 = W_ST + 3 * 54
W_JUNK = W_L2 + 54
W_SUB = W_JUNK + 1
PR_ROWS = 27 * M
SR = 4384


def _expand(vals):
    n = len(vals)
    if n == 1:
        return [vals[0]]
    h = n // 2
    lo, hi = vals[:h], vals[h:]
    return _expand(lo) + _expand([a + b for a, b in zip(lo, hi)]) + _expand(hi)


def _pure_idx(k):
    if k == 0:
        return [0]
    sub = _pure_idx(k - 1)
    h = 2 ** (k - 1)
    return list(sub) + [None] * len(sub) + [None if i is None else i + h for i in sub]


PURE = _pure_idx(3)


def _in_expand(seq, n):
    if n == 1:
        return [seq[0]]
    h = n // 2
    mid = seq[h:3 * h - 1]
    lo = [a - b for a, b in zip(seq[0:2 * h - 1], mid)]
    out = _in_expand(lo, h)
    out += _in_expand(mid, h)
    hi = [a - b for a, b in zip(seq[2 * h:4 * h - 1], mid)]
    out += _in_expand(hi, h)
    return out


def _out_combine(get, base, n):
    if n == 1:
        return [get(base)]
    t = 1
    while 2 * t < n + 1 and t < n:
        break
    third = 3 ** ((n.bit_length() - 1) - 1)
    lo = _out_combine(get, base, n // 2)
    s = _out_combine(get, base + third, n // 2)
    out = [a + b for a, b in zip(s, lo)]
    hi = _out_combine(get, base + 2 * third, n // 2)
    out += [a + b for a, b in zip(s, hi)]
    return out


def _gelu(x):
    c0 = 0.7978845608028654
    c1 = c0 * 0.044715
    inner = x * (c0 + c1 * (x * x))
    hx = 0.5 * x
    return hx + hx * jnp.tanh(inner)


class _Alloc:
    def __init__(self):
        self.fill = []

    def __call__(self, n):
        for s, f in enumerate(self.fill):
            if f + n <= SR:
                self.fill[s] += n
                return (s, f)
        self.fill.append(n)
        return (len(self.fill) - 1, 0)


_al = _Alloc()
XP_LOC = [_al(NCH * XP_ROWS) for _ in range(B)]
PR1_LOC = [[_al(PR_ROWS) for _ in range(3)] for _ in range(2)]
PR2_LOC = [_al(PR_ROWS) for _ in range(2)]
HB_LOC = [_al(HB_ROWS) for _ in range(NCH)]
JA_LOC = _al(64)
NSLOT_A = len(_al.fill)

G_LO, G_S, G_HI = 0, 1, 2

_PROFILE = False


class _NoScope:
    def __enter__(self):
        return self

    def __exit__(self, *a):
        return False


def _scope(name):
    return jax.named_scope(name) if _PROFILE else _NoScope()


def _kernel(x_hbm, w1_hbm, w2_hbm, g_hbm, wf_hbm, wg_hbm, wo_hbm, out_hbm,
            aw, aa, lhs1, xin, gin, wf, wg, wo,
            fbuf, fe, ge, obuf, zs, sems, osems):
    stages = [W_ST, W_ST + 54, W_ST + 108]
    aw16 = aw.bitcast(BF16)

    def wcopy(conv, nc, g):
        src = w1_hbm if conv == 0 else w2_hbm
        nt = 16 if g == 0 else 15
        slot = conv * 8 + nc * 2 + g
        return pltpu.make_async_copy(
            src.at[pl.ds(16 * g, nt), :, pl.ds(nc * NL, NL)],
            aw16.at[pl.ds(16 * slot, nt)], sems.at[slot])

    cp_x = pltpu.make_async_copy(x_hbm, xin, sems.at[16])
    cp_g = pltpu.make_async_copy(g_hbm, gin, sems.at[17])
    cp_wg = pltpu.make_async_copy(wg_hbm, wg, sems.at[18])
    cp_wf = pltpu.make_async_copy(wf_hbm, wf, sems.at[19])
    cp_wo = pltpu.make_async_copy(wo_hbm, wo, sems.at[20])

    cp_x.start()
    for nc in range(NCH):
        for g in range(2):
            wcopy(0, nc, g).start()
    cp_g.start()
    cp_wg.start()
    cp_wf.start()
    for nc in range(NCH):
        for g in range(2):
            wcopy(1, nc, g).start()
    cp_wo.start()

    for conv in range(2):
        for nc in range(NCH):
            aw[16 * (conv * 8 + nc * 2 + 1) + 15] = jnp.zeros((256, NL), U32)
    for b in range(B):
        s, o = XP_LOC[b]
        for lt in range(NCH):
            r0 = o + lt * XP_ROWS
            aa[s, r0:r0 + 16, :] = jnp.zeros((16, NL), F32)
            aa[s, r0 + 33 * 31 + 24:r0 + 33 * 33, :] = jnp.zeros((33 * 2 - 24, NL), F32)
    for lt in range(NCH):
        s, o = HB_LOC[lt]
        for blk in range(17):
            aa[s, o + blk * HB_BLK:o + blk * HB_BLK + 16, :] = jnp.zeros((16, NL), F32)

    zbox = []

    with _scope("p_xwait"):
        cp_x.wait()
    with _scope("p_xconv"):
        for b in range(B):
            s, o = XP_LOC[b]
            for lt in range(NCH):
                r0 = o + lt * XP_ROWS
                for gq in range(32):
                    t0, t1 = max(32 * gq - 16, 0), min(32 * gq + 16, T)
                    d0 = r0 + 33 * gq + (t0 - (32 * gq - 16))
                    aa[s, d0:d0 + (t1 - t0), :] = xin[b, t0:t1, lt * NL:(lt + 1) * NL].astype(F32)

    def pack2(a, b):
        return pltpu.pack_elementwise([a, b], packed_dtype=BF16).astype(U32)

    def lhs1_block(gi):
        def body(i, carry):
            ag = i // 8
            kt = i % 8
            e = kt // 4
            lt = kt % 4
            base = lt * XP_ROWS + 33 * 8 * ag + e
            lvs = []
            for b in range(B):
                def ld(u):
                    off = 2 * u + 1 + (1 if u >= 16 else 0)
                    if u == 15:
                        return aa[XP_LOC[b][0], pl.ds(XP_LOC[b][1] + base + e + off, 8, stride=33), :]
                    return aa[XP_LOC[b][0], pl.ds(XP_LOC[b][1] + base + off, 8, stride=33), :]
                if gi == G_S:
                    seq = [ld(8 + j) for j in range(15)]
                elif gi == G_LO:
                    seq = [ld(j) - ld(8 + j) for j in range(15)]
                else:
                    seq = [ld(16 + j) - ld(8 + j) for j in range(15)]
                lvs.append(_in_expand(seq, 8))
            row = pl.multiple_of(ag * 8, 8)
            for c in range(27):
                lhs1[gi * 27 + c, kt, pl.ds(row, 8), :] = pack2(lvs[0][c], lvs[1][c])
            return carry
        jax.lax.fori_loop(0, 32, body, 0)

    def unpack(v, h):
        return pltpu.unpack_elementwise(v, index=h, packed_dtype=BF16, unpacked_dtype=F32)

    def t_load(zz, slots, e, r):
        return [[aw[zz + 16 * sl + 2 * m + e, pl.ds(r, 8), :] for m in range(8)] for sl in slots]

    def t_comp(raws, st, e, r):
        lvs = []
        for h in range(2):
            if len(raws) == 2:
                src = [unpack(a, h) + unpack(b, h) for a, b in zip(*raws)]
            else:
                src = [unpack(a, h) for a in raws[0]]
            lvs.append(_expand(src))
        for c in range(27):
            if PURE[c] is None or len(raws) == 2:
                aw[st + 2 * c + e, pl.ds(r, 8), :] = pack2(lvs[0][c], lvs[1][c])

    def t_items(slots, st):
        return [((lambda e=e, r=r: t_load(zbox[0], slots, e, r)),
                 (lambda raws, e=e, r=r: t_comp(raws, st, e, r)))
                for e in range(2) for r in range(0, 256, 8)]

    def d_items(nc):
        par = nc % 2
        hs, ho = HB_LOC[nc]

        def item(rb, k):
            sS, oS = PR1_LOC[par][G_S]
            sK, oK = PR1_LOC[par][G_LO if k == 0 else G_HI]

            def get(c):
                r = c * M + rb * 8
                return aa[zbox[0] + sS, oS + r:oS + r + 8, :] + aa[zbox[0] + sK, oK + r:oK + r + 8, :]
            ys = _out_combine(get, 0, 8)
            for r_ in range(8):
                p = 8 * k + r_
                y = _gelu(ys[r_])
                if rb == 7 and p >= 4:
                    rows = jax.lax.broadcasted_iota(jnp.int32, (8, NL), 0)
                    y = jnp.where(rows < 6, y, 0.0)
                r0 = ho + p * HB_BLK + 16 + rb * 8
                aa[hs, r0:r0 + 8, :] = y
        return [(None, (lambda _, rb=rb, k=k: item(rb, k))) for rb in range(8) for k in range(2)]

    def e_items(nc):
        hs, ho = HB_LOC[nc]

        def item(j, e, ag, br):
            a0 = 8 * ag
            lvs = []
            for b in range(B):
                def ld(u):
                    q = 2 * (8 * j + u) + e
                    p = (q - 15) % 16
                    c = (q - 15) // 16
                    r0 = ho + p * HB_BLK + 16 + 2 * (a0 + c) + b
                    return aa[zbox[0] + hs, pl.ds(r0, 8, stride=2), :]
                mid = [ld(4 + i) for i in range(7)]
                if br == 1:
                    seq = mid
                elif br == 0:
                    seq = [(ld(i) if i < 4 else mid[i - 4]) - mid[i] for i in range(7)]
                else:
                    seq = [(ld(8 + i) if i >= 3 else mid[4 + i]) - mid[i] for i in range(7)]
                lvs.append(_in_expand(seq, 4))
            kt = e * 4 + nc
            for c in range(9):
                aw[W_L2 + j * 27 + br * 9 + c, kt * 32 + a0:kt * 32 + a0 + 8, :] = pack2(lvs[0][c], lvs[1][c])
        return [(None, (lambda _, j=j, e=e, ag=ag, br=br: item(j, e, ag, br)))
                for j in range(2) for e in range(2) for ag in range(4) for br in range(3)]

    def f_items(nc):
        s2, o2 = PR2_LOC[nc % 2]

        def item(rb):
            def get(c):
                r = o2 + c * M + rb * 8
                return aa[zbox[0] + s2, r:r + 8, :]
            ys = _out_combine(get, 0, 8)
            for p in range(8):
                fbuf[nc, p * M + rb * 8:p * M + rb * 8 + 8, :] = _gelu(ys[p]).astype(BF16)
        return [(None, (lambda _, rb=rb: item(rb))) for rb in range(8)]

    cnt = [0]

    def pace(v, wa=True):
        u = cnt[0] % 8
        cnt[0] += 1
        aw[W_JUNK, 8 * u:8 * u + 8, :] = pltpu.bitcast(v, U32)
        if wa:
            aa[JA_LOC[0], JA_LOC[1] + 8 * u:JA_LOC[1] + 8 * u + 8, :] = v

    def leaf_units(lhs_get, st, slot, pure_ok, ploc, accumulate):
        units = []
        state = {}
        ps, po = ploc
        for c in range(27):
            for e in range(2):
                def unit(c=c, e=e):
                    if pure_ok and PURE[c] is not None:
                        w = aw[16 * slot + 2 * PURE[c] + e]
                    else:
                        w = aw[st + 2 * c + e]
                    w = pltpu.bitcast(w, BF16)
                    l = jnp.concatenate(
                        [pltpu.bitcast(lhs_get(c, e * 4 + k), BF16) for k in range(4)], axis=1)
                    res = jnp.dot(l, w, preferred_element_type=F32)
                    r = po + c * M
                    if e == 0:
                        if accumulate:
                            res = res + aa[ps, r:r + M, :]
                        state[c] = res
                        pace(res[M - 8:M])
                    else:
                        res = res + state.pop(c)
                        aa[ps, r:r + M, :] = res
                        pace(res[M - 8:M], wa=False)
                units.append(unit)
        return units

    def run_step(units, groups, name):
        with _scope(name):
            run_step_(units, groups)

    def run_step_(units, groups):
        seq = []
        for pre, items in groups:
            for i, it in enumerate(items):
                seq.append((pre if i == 0 else None, it))
        nu, ni = len(units), len(seq)
        loaded = {}

        def preload(k):
            if k < ni and k not in loaded:
                pre, (ld, _) = seq[k]
                if pre is not None:
                    pre()
                loaded[k] = ld() if ld is not None else None

        k = 0
        for u, unit in enumerate(units):
            unit()
            upto = ni * (u + 1) // nu
            while k < upto:
                preload(k)
                preload(k + 1)
                seq[k][1][1](loaded.pop(k))
                k += 1

    with _scope("p_lhs1"):
        lhs1_block(G_LO)
        lhs1_block(G_HI)
        lhs1_block(G_S)

    with _scope("p_wwait"):
        wcopy(0, 0, 0).wait()

    def t0_body(i, carry):
        e = i // 32
        r = pl.multiple_of((i % 32) * 8, 8)
        t_comp(t_load(0, [0], e, r), stages[G_LO], e, r)
        zs[0] = i // 64
        return carry
    with _scope("p_t0"):
        jax.lax.fori_loop(0, 64, t0_body, 0)
    zbox.append(zs[0])

    def l1get(gi):
        return lambda c, kt: lhs1[gi * 27 + c, kt]

    for nc in range(NCH):
        par = nc % 2
        slo, shi = nc * 2, nc * 2 + 1
        groups = []
        if nc > 0:
            groups.append((None, d_items(nc - 1)))
        groups.append((wcopy(0, nc, 1).wait, t_items([shi], stages[G_HI])))
        run_step(leaf_units(l1get(G_LO), stages[G_LO], slo, True, PR1_LOC[par][G_LO], False), groups, "c1_lo%d" % nc)
        run_step(leaf_units(l1get(G_HI), stages[G_HI], shi, True, PR1_LOC[par][G_HI], False),
                 [(None, t_items([slo, shi], stages[G_S]))], "c1_hi%d" % nc)
        groups = []
        if nc > 0:
            groups.append((None, e_items(nc - 1)))
        if nc + 1 < NCH:
            groups.append((wcopy(0, nc + 1, 0).wait, t_items([slo + 2], stages[G_LO])))
        else:
            groups.append((wcopy(1, 0, 0).wait, t_items([8], stages[G_LO])))
        run_step(leaf_units(l1get(G_S), stages[G_S], None, False, PR1_LOC[par][G_S], False), groups, "c1_S%d" % nc)

    with _scope("c1_tail"):
        for _, it in d_items(NCH - 1):
            it(None)
        for _, it in e_items(NCH - 1):
            it(None)

    cp_g.wait()
    cp_wg.wait()
    cp_wf.wait()
    ge[...] = jnp.dot(gin[...], wg[...], preferred_element_type=F32)

    def l2get(j):
        return lambda c, kt: aw[W_L2 + j * 27 + c, kt * 32:(kt + 1) * 32, :]

    def fe_unit(kc):
        def unit():
            res = jnp.dot(fbuf[kc], wf[kc * NL:(kc + 1) * NL, :], preferred_element_type=F32)
            for lt in range(NCH):
                if kc == 0:
                    fe[lt] = res[:, lt * NL:(lt + 1) * NL]
                else:
                    fe[lt] += res[:, lt * NL:(lt + 1) * NL]
        return unit

    for nc in range(NCH):
        par = nc % 2
        slo, shi = 8 + nc * 2, 8 + nc * 2 + 1
        groups = []
        if nc > 0:
            groups.append((None, f_items(nc - 1)))
        groups.append((wcopy(1, nc, 1).wait, t_items([shi], stages[G_HI])))
        run_step(leaf_units(l2get(0), stages[G_LO], slo, True, PR2_LOC[par], False), groups, "c2_lo%d" % nc)
        units = leaf_units(l2get(1), stages[G_HI], shi, True, PR2_LOC[par], True)
        if nc > 0:
            units = units[:27] + [fe_unit(nc - 1)] + units[27:]
        groups = []
        if nc + 1 < NCH:
            groups.append((wcopy(1, nc + 1, 0).wait, t_items([slo + 2], stages[G_LO])))
        run_step(units, groups, "c2_hi%d" % nc)

    with _scope("c2_tail"):
        for _, it in f_items(NCH - 1):
            it(None)
        fe_unit(NCH - 1)()

    cp_wo.wait()

    def ocopy(ch):
        b, ck = ch // 4, ch % 4
        n = 512 if ck < 3 else 464
        return pltpu.make_async_copy(
            obuf.at[ch % 2, pl.ds(0, n)],
            out_hbm.at[pl.ds((b * 250 + 64 * ck) * 8, n)], osems.at[ch % 2])

    for ch in range(8):
      with _scope("joint%d" % ch):
        b, ck = ch // 4, ch % 4
        geb = ge[b * 8:(b + 1) * 8, :]
        parts = []
        for i in range(8):
            a2 = 8 * ck + i
            nt = 2 if a2 == 31 else 8
            ft = jnp.concatenate(
                [fe[lt, pl.ds(2 * a2 + b, nt, stride=M), :] for lt in range(NCH)], axis=1)
            jj = jnp.tanh(ft[:, None, :] + geb[None, :, :])
            parts.append(jj.reshape(nt * 8, D).astype(BF16))
        jv = jnp.concatenate(parts, axis=0)
        n = jv.shape[0]
        res = jnp.dot(jv, wo[...], preferred_element_type=F32)
        if ch >= 2:
            ocopy(ch - 2).wait()
        obuf[ch % 2, 0:n, :] = res.astype(BF16)
        ocopy(ch).start()
    ocopy(6).wait()
    ocopy(7).wait()


@jax.jit
def pallas_standalone__seq2seq_rnn_t_joint__speech_kernel(
    x: jax.Array,
    w1: jax.Array,
    w2: jax.Array,
    g: jax.Array,
    w_f: jax.Array,
    w_g: jax.Array,
    w_o: jax.Array,
):
    any_spec = pl.BlockSpec(memory_space=pl.ANY)
    out = pl.pallas_call(
        _kernel,
        out_shape=jax.ShapeDtypeStruct((B * 250 * NU, D), BF16),
        in_specs=[any_spec] * 7,
        out_specs=any_spec,
        scratch_shapes=[
            pltpu.VMEM((W_SUB, 256, NL), U32),
            pltpu.VMEM((NSLOT_A, SR, NL), F32),
            pltpu.VMEM((81, 8, M // 2, NL), U32),
            pltpu.VMEM((B, T, D), BF16),
            pltpu.VMEM((B * NU, D), BF16),
            pltpu.VMEM((D, D), BF16),
            pltpu.VMEM((D, D), BF16),
            pltpu.VMEM((D, D), BF16),
            pltpu.VMEM((NCH, 512, NL), BF16),
            pltpu.VMEM((NCH, 512, NL), F32),
            pltpu.VMEM((B * NU, D), F32),
            pltpu.VMEM((2, 512, D), BF16),
            pltpu.SMEM((1,), jnp.int32),
            pltpu.SemaphoreType.DMA((21,)),
            pltpu.SemaphoreType.DMA((2,)),
        ],
        compiler_params=pltpu.CompilerParams(vmem_limit_bytes=120 * 1024 * 1024),
    )(x, w1, w2, g.reshape(B * NU, D), w_f, w_g, w_o)
    return out.reshape(B, 250, NU, D)
```

```python
import jax
import jax.numpy as jnp
import jax.experimental.pallas as pl
import jax.experimental.pallas.tpu as pltpu

F32 = jnp.float32
BF16 = jnp.bfloat16
U32 = jnp.uint32

B, T, D, KT, NU = 2, 1000, 512, 31, 8
NL = 128
NCH = D // NL
M = 64
XP_ROWS = 1096
HB_BLK = 80
HB_ROWS = 16 * HB_BLK + 16
W_JUNK = 256
W_SUB = W_JUNK + 1
PR_ROWS = 27 * M
SR = 4384


class _Lazy:
    def __init__(self, fn):
        self.fn = fn
        self.v = None

    def get(self):
        if self.v is None:
            self.v = self.fn()
        return self.v


def _expand(vals, emit, base=0):
    n = len(vals)
    if n == 1:
        emit(base, vals[0])
        return
    h = n // 2
    third = 3 ** (h.bit_length() - 1)
    lo, hi = vals[:h], vals[h:]
    _expand(lo, emit, base)

    def add(a, b):
        return _Lazy(lambda: (a.get()[0] + b.get()[0], a.get()[1] + b.get()[1]))
    _expand([add(a, b) for a, b in zip(lo, hi)], emit, base + third)
    _expand(hi, emit, base + 2 * third)


def _pure_idx(k):
    if k == 0:
        return [0]
    sub = _pure_idx(k - 1)
    h = 2 ** (k - 1)
    return list(sub) + [None] * len(sub) + [None if i is None else i + h for i in sub]


PURE = _pure_idx(3)


def _in_expand(seq, n, emit, base=0):
    if n == 1:
        emit(base, seq[0])
        return
    h = n // 2
    third = 3 ** (h.bit_length() - 1)
    mid = seq[h:3 * h - 1]
    _in_expand([(a[0] - b[0], a[1] - b[1]) for a, b in zip(seq[0:2 * h - 1], mid)], h, emit, base)
    _in_expand(mid, h, emit, base + third)
    _in_expand([(a[0] - b[0], a[1] - b[1]) for a, b in zip(seq[2 * h:4 * h - 1], mid)], h, emit,
               base + 2 * third)


def _out_combine(get, base, n):
    if n == 1:
        return [get(base)]
    third = 3 ** ((n.bit_length() - 1) - 1)
    lo = _out_combine(get, base, n // 2)
    s = _out_combine(get, base + third, n // 2)
    out = [a + b for a, b in zip(s, lo)]
    hi = _out_combine(get, base + 2 * third, n // 2)
    out += [a + b for a, b in zip(s, hi)]
    return out


def _gelu(x):
    c0 = 0.7978845608028654
    c1 = c0 * 0.044715
    inner = x * (c0 + c1 * (x * x))
    hx = 0.5 * x
    return hx + hx * jnp.tanh(inner)


class _Alloc:
    def __init__(self):
        self.fill = []

    def __call__(self, n):
        for s, f in enumerate(self.fill):
            if f + n <= SR:
                self.fill[s] += n
                return (s, f)
        self.fill.append(n)
        return (len(self.fill) - 1, 0)


_al = _Alloc()
XP_LOC = [_al(NCH * XP_ROWS) for _ in range(B)]
PR1_LOC = [[_al(PR_ROWS) for _ in range(3)] for _ in range(2)]
PR2_LOC = [_al(PR_ROWS) for _ in range(2)]
HB_LOC = [_al(HB_ROWS) for _ in range(NCH)]
JA_LOC = _al(64)
NSLOT_A = len(_al.fill)

G_LO, G_S, G_HI = 0, 1, 2

_PROFILE = False
TOKEN_LAG = 2


class _NoScope:
    def __enter__(self):
        return self

    def __exit__(self, *a):
        return False


def _scope(name):
    return jax.named_scope(name) if _PROFILE else _NoScope()


def _kernel(x_hbm, w1_hbm, w2_hbm, g_hbm, wf_hbm, wg_hbm, wo_hbm, out_hbm,
            aw, st0, st1, st2, l2a, l2b, aa, lhs1, xin, gin, wf, wg, wo,
            fbuf, fe, ge, obuf, zs, sems, osems):
    stages = [st0, st1, st2]
    aw16 = aw.bitcast(BF16)

    def wcopy(conv, nc, g):
        src = w1_hbm if conv == 0 else w2_hbm
        nt = 16 if g == 0 else 15
        slot = conv * 8 + nc * 2 + g
        return pltpu.make_async_copy(
            src.at[pl.ds(16 * g, nt), :, pl.ds(nc * NL, NL)],
            aw16.at[pl.ds(16 * slot, nt)], sems.at[slot])

    cp_x = [pltpu.make_async_copy(x_hbm.at[b], xin.at[b], sems.at[(16, 21)[b]]) for b in range(B)]
    cp_g = pltpu.make_async_copy(g_hbm, gin, sems.at[17])
    cp_wg = pltpu.make_async_copy(wg_hbm, wg, sems.at[18])
    cp_wf = pltpu.make_async_copy(wf_hbm, wf, sems.at[19])
    cp_wo = pltpu.make_async_copy(wo_hbm, wo, sems.at[20])

    for b in range(B):
        cp_x[b].start()
    for nc in range(NCH):
        for g in range(2):
            wcopy(0, nc, g).start()
    cp_g.start()
    cp_wg.start()
    cp_wf.start()
    for nc in range(NCH):
        for g in range(2):
            wcopy(1, nc, g).start()
    cp_wo.start()

    for conv in range(2):
        for nc in range(NCH):
            aw[16 * (conv * 8 + nc * 2 + 1) + 15] = jnp.zeros((256, NL), U32)
    for b in range(B):
        s, o = XP_LOC[b]
        for lt in range(NCH):
            r0 = o + lt * XP_ROWS
            aa[s, r0:r0 + 16, :] = jnp.zeros((16, NL), F32)
            aa[s, r0 + 33 * 31 + 24:r0 + 33 * 33, :] = jnp.zeros((33 * 2 - 24, NL), F32)
    for lt in range(NCH):
        s, o = HB_LOC[lt]
        for blk in range(17):
            aa[s, o + blk * HB_BLK:o + blk * HB_BLK + 16, :] = jnp.zeros((16, NL), F32)

    zbox = []

    with _scope("p_xconv"):
        for b in range(B):
            cp_x[b].wait()
            s, o = XP_LOC[b]
            for lt in range(NCH):
                r0 = o + lt * XP_ROWS
                for gq in range(32):
                    t0, t1 = max(32 * gq - 16, 0), min(32 * gq + 16, T)
                    d0 = r0 + 33 * gq + (t0 - (32 * gq - 16))
                    aa[s, d0:d0 + (t1 - t0), :] = xin[b, t0:t1, lt * NL:(lt + 1) * NL].astype(F32)

    def pack2(a, b):
        return pltpu.pack_elementwise([a, b], packed_dtype=BF16).astype(U32)

    def lhs1_all():
        def body(i, carry):
            ag = i // 8
            kt = i % 8
            e = kt // 4
            lt = kt % 4
            base = lt * XP_ROWS + 33 * 8 * ag + e
            row = pl.multiple_of(ag * 8, 8)

            def ld(b, u):
                off = XP_LOC[b][1] + base + 2 * u + 1 + (1 if u >= 16 else 0)
                if u == 15:
                    off = off + e
                return aa[XP_LOC[b][0], pl.ds(off, 8, stride=33), :]

            for gi in (G_LO, G_HI, G_S):
                if gi == G_S:
                    seq = [tuple(ld(b, 8 + j) for b in range(B)) for j in range(15)]
                elif gi == G_LO:
                    seq = [tuple(ld(b, j) - ld(b, 8 + j) for b in range(B)) for j in range(15)]
                else:
                    seq = [tuple(ld(b, 16 + j) - ld(b, 8 + j) for b in range(B)) for j in range(15)]

                def put(c, v, gi=gi):
                    lhs1[gi * 27 + c, kt, pl.ds(row, 8), :] = pack2(v[0], v[1])
                _in_expand(seq, 8, put)
            zs[0] = i // 32
            return carry
        jax.lax.fori_loop(0, 32, body, 0)

    def unpack(v, h):
        return pltpu.unpack_elementwise(v, index=h, packed_dtype=BF16, unpacked_dtype=F32)

    def t_pos(slots, st, e, r):
        def fetch(m):
            raw = [aw[zbox[0] + 16 * sl + 2 * m + e, pl.ds(r, 8), :] for sl in slots]
            if len(slots) == 2:
                return tuple(unpack(raw[0], h) + unpack(raw[1], h) for h in range(2))
            return tuple(unpack(raw[0], h) for h in range(2))
        src = [_Lazy(lambda m=m: fetch(m)) for m in range(8)]

        def put(c, v):
            if PURE[c] is None or len(slots) == 2:
                v = v.get()
                st[2 * c + e, pl.ds(r, 8), :] = pack2(v[0], v[1])
        _expand(src, put)
        last = 26 if len(slots) == 2 else 25
        return lambda: st[zbox[0] + 2 * last + e, pl.ds(r, 8), :]

    def t_items(slots, st):
        return [(None, (lambda _, e=e, r=r: t_pos(slots, st, e, r)))
                for e in range(2) for r in range(0, 256, 8)]

    def d_items(nc):
        par = nc % 2
        hs, ho = HB_LOC[nc]

        def item(rb, k):
            sS, oS = PR1_LOC[par][G_S]
            sK, oK = PR1_LOC[par][G_LO if k == 0 else G_HI]

            def get(c):
                r = c * M + rb * 8
                return aa[zbox[0] + sS, oS + r:oS + r + 8, :] + aa[zbox[0] + sK, oK + r:oK + r + 8, :]
            ys = _out_combine(get, 0, 8)
            for r_ in range(8):
                p = 8 * k + r_
                y = _gelu(ys[r_])
                if rb == 7 and p >= 4:
                    rows = jax.lax.broadcasted_iota(jnp.int32, (8, NL), 0)
                    y = jnp.where(rows < 6, y, 0.0)
                r0 = ho + p * HB_BLK + 16 + rb * 8
                aa[hs, r0:r0 + 8, :] = y
        return [(None, (lambda _, rb=rb, k=k: item(rb, k))) for rb in range(8) for k in range(2)]

    def l2loc(kt):
        e, lt = kt // 4, kt % 4
        if lt == 3:
            return l2b, e * 32
        return l2a, (e * 3 + lt) * 32

    def e_items(nc):
        hs, ho = HB_LOC[nc]

        def item(j, e, ag, br):
            a0 = 8 * ag

            def ld(u):
                q = 2 * (8 * j + u) + e
                p = (q - 15) % 16
                c = (q - 15) // 16
                r0 = ho + p * HB_BLK + 16 + 2 * (a0 + c)
                return tuple(aa[zbox[0] + hs, pl.ds(r0 + b, 8, stride=2), :] for b in range(B))

            def sub(a, b):
                return (a[0] - b[0], a[1] - b[1])
            mid = [ld(4 + i) for i in range(7)]
            if br == 1:
                seq = mid
            elif br == 0:
                seq = [sub(ld(i) if i < 4 else mid[i - 4], mid[i]) for i in range(7)]
            else:
                seq = [sub(ld(8 + i) if i >= 3 else mid[4 + i], mid[i]) for i in range(7)]
            l2, r0 = l2loc(e * 4 + nc)

            def put(c, v):
                l2[j * 27 + br * 9 + c, r0 + a0:r0 + a0 + 8, :] = pack2(v[0], v[1])
            _in_expand(seq, 4, put)
            return lambda: l2[zbox[0] + j * 27 + br * 9 + 8, r0 + a0:r0 + a0 + 8, :]
        return [(None, (lambda _, j=j, e=e, ag=ag, br=br: item(j, e, ag, br)))
                for j in range(2) for e in range(2) for ag in range(4) for br in range(3)]

    def f_items(nc):
        s2, o2 = PR2_LOC[nc % 2]

        def item(rb):
            def get(c):
                r = o2 + c * M + rb * 8
                return aa[zbox[0] + s2, r:r + 8, :]
            ys = _out_combine(get, 0, 8)
            for p in range(8):
                fbuf[nc, p * M + rb * 8:p * M + rb * 8 + 8, :] = _gelu(ys[p]).astype(BF16)
        return [(None, (lambda _, rb=rb: item(rb))) for rb in range(8)]

    cnt = [0]

    no_pace_w = [False, 0]
    tokens = []

    def pace(v, wa=True):
        u = cnt[0] % 8
        cnt[0] += 1
        if not no_pace_w[0]:
            val = pltpu.bitcast(v, U32)
            while tokens and tokens[0][0] <= no_pace_w[1]:
                val = val ^ tokens.pop(0)[1]()
            aw[W_JUNK, 8 * u:8 * u + 8, :] = val
        if wa:
            aa[JA_LOC[0], JA_LOC[1] + 8 * u:JA_LOC[1] + 8 * u + 8, :] = v

    def leaf_units(lhs_get, st, slot, pure_ok, ploc, accumulate, order=None, lts=(0, 4)):
        units = []
        state = {}
        ps, po = ploc
        l0, l1 = lts

        def half(c, e):
            if pure_ok and PURE[c] is not None:
                w = aw[16 * slot + 2 * PURE[c] + e, 64 * l0:64 * l1, :]
            else:
                w = st[zbox[0] + 2 * c + e, 64 * l0:64 * l1, :]
            w = pltpu.bitcast(w, BF16)
            l = [pltpu.bitcast(lhs_get(c, e * 4 + k), BF16) for k in range(l0, l1)]
            l = jnp.concatenate(l, axis=1) if len(l) > 1 else l[0]
            return jnp.dot(l, w, preferred_element_type=F32)

        for c in (order if order is not None else range(27)):
            r = po + c * M
            if l1 - l0 >= 2:
                def unit0(c=c, r=r):
                    res = half(c, 0)
                    if accumulate:
                        res = res + aa[ps, r:r + M, :]
                    state[c] = res
                    pace(res[M - 8:M])

                def unit1(c=c, r=r):
                    res = half(c, 1) + state.pop(c)
                    aa[ps, r:r + M, :] = res
                    pace(res[M - 8:M], wa=False)
                units += [(unit0, l1 - l0), (unit1, l1 - l0)]
            else:
                def unit01(c=c, r=r):
                    res = half(c, 0) + half(c, 1)
                    if accumulate:
                        res = res + aa[ps, r:r + M, :]
                    aa[ps, r:r + M, :] = res
                    pace(res[M - 8:M], wa=False)
                units.append((unit01, 2 * (l1 - l0)))
        return units

    tl_units = []
    tl_items = []

    def now():
        return float(sum(w for _, w in tl_units))

    def add_units(us):
        tl_units.extend(us)

    def add_stream(items, t0, t1, pre=None):
        n = len(items)
        for i, (ld, comp) in enumerate(items):
            tl_items.append((t0 + (i + 0.5) * (t1 - t0) / n, len(tl_items),
                             pre if i == 0 else None, ld, comp))

    def emit():
        seq = sorted(tl_items, key=lambda it: (it[0], it[1]))
        loaded = {}

        def preload(k):
            if k < len(seq) and k not in loaded:
                _, _, pre, ld, _ = seq[k]
                if pre is not None:
                    pre()
                loaded[k] = ld() if ld is not None else None

        ends = []
        t = 0.0
        for _, w in tl_units:
            t += w
            ends.append(t)
        quiet = set()
        for it in seq:
            if it[2] is not None:
                u = next(i for i, e in enumerate(ends) if it[0] < e)
                quiet.update((u, u - 1))
        k = 0
        for u, (fn, w) in enumerate(tl_units):
            no_pace_w[0] = u in quiet
            no_pace_w[1] = u
            fn()
            t = ends[u]
            while k < len(seq) and seq[k][0] < t:
                preload(k)
                if k + 1 < len(seq) and seq[k + 1][0] < t and seq[k + 1][2] is None:
                    preload(k + 1)
                tk = seq[k][4](loaded.pop(k))
                if tk is not None:
                    tokens.append((u + TOKEN_LAG, tk))
                k += 1
        no_pace_w[0] = False
        assert k == len(seq)

    with _scope("p_lhs1"):
        lhs1_all()
    zbox.append(zs[0])

    def l1get(gi):
        return lambda c, kt: lhs1[gi * 27 + c, kt]

    def l2get(j):
        def get(c, kt):
            l2, r0 = l2loc(kt)
            return l2[zbox[0] + j * 27 + c, r0:r0 + 32, :]
        return get

    def fe_unit(kc):
        def unit():
            res = jnp.dot(fbuf[kc], wf[kc * NL:(kc + 1) * NL, :], preferred_element_type=F32)
            for lt in range(NCH):
                if kc == 0:
                    fe[lt] = res[:, lt * NL:(lt + 1) * NL]
                else:
                    fe[lt] += res[:, lt * NL:(lt + 1) * NL]
        return (unit, 32)

    def waits(*cps):
        def go():
            for cp in cps:
                cp.wait()
        return go

    def ge_unit():
        res = jnp.dot(gin[...], wg[...], preferred_element_type=F32)
        for lt in range(NCH):
            ge[lt, 32:48, :] = res[:, lt * NL:(lt + 1) * NL]
        for lt in range(NCH):
            for b in range(B):
                for par in range(2):
                    v = ge[lt, pl.ds(32 + 8 * b + par, 4, stride=2), :]
                    ge[lt, 16 * b + 8 * par:16 * b + 8 * par + 4, :] = v
                    ge[lt, 16 * b + 8 * par + 4:16 * b + 8 * par + 8, :] = v

    pure_first = ([c for c in range(27) if PURE[c] is not None]
                  + [c for c in range(27) if PURE[c] is None])
    STEP = 54 * 4.0

    wcopy(0, 0, 0).wait()
    for nc in range(NCH):
        par = nc % 2
        slo, shi = nc * 2, nc * 2 + 1
        t = now()
        if nc == 0:
            add_stream(t_items([slo], stages[G_LO]), t, t + 60)
            add_stream(t_items([shi], stages[G_HI]), t + 140, t + STEP + 56, wcopy(0, nc, 1).wait)
            add_stream(t_items([slo, shi], stages[G_S]), t + STEP + 56, t + 2 * STEP - 12)
        else:
            add_stream(t_items([shi], stages[G_HI]), t - 44, t + 139,
                       wcopy(0, nc, 1).wait if nc < 2 else None)
            add_stream(t_items([slo, shi], stages[G_S]), t + 139, t + 2 * STEP - 12)
            add_stream(d_items(nc - 1), t, t + 330)
            add_stream(e_items(nc - 1), t + 330, t + 3 * STEP - 44)
        if nc + 1 < NCH:
            add_stream(t_items([slo + 2], stages[G_LO]), t + 2 * STEP - 12, t + 3 * STEP - 44,
                       wcopy(0, nc + 1, 0).wait if nc < 1 else
                       waits(wcopy(0, nc + 1, 0), wcopy(0, nc + 1, 1)))
        else:
            add_stream(t_items([8], stages[G_LO]), t + 2 * STEP - 12, t + 3 * STEP,
                       waits(cp_g, cp_wg, cp_wf, wcopy(1, 0, 0), wcopy(1, 0, 1), wcopy(1, 1, 0)))
        add_units(leaf_units(l1get(G_LO), stages[G_LO], slo, True, PR1_LOC[par][G_LO], False,
                             order=pure_first))
        add_units(leaf_units(l1get(G_HI), stages[G_HI], shi, True, PR1_LOC[par][G_HI], False,
                             order=pure_first))
        add_units(leaf_units(l1get(G_S), stages[G_S], None, False, PR1_LOC[par][G_S], False))

    for nc in range(NCH):
        par = nc % 2
        slo, shi = 8 + nc * 2, 8 + nc * 2 + 1
        t = now()
        if nc == 0:
            add_stream(d_items(NCH - 1), t, t + 0.3 * STEP)
            add_stream(e_items(NCH - 1), t + 0.3 * STEP, t + 0.72 * STEP)
            add_stream(t_items([shi], stages[G_HI]), t, t + STEP + 32)
            add_units(leaf_units(l2get(0), stages[G_LO], slo, True, PR2_LOC[par], False, lts=(0, 3),
                                 order=pure_first))
            add_units(leaf_units(l2get(0), stages[G_LO], slo, True, PR2_LOC[par], True, lts=(3, 4)))
        else:
            add_stream(f_items(nc - 1), t, t + STEP)
            add_stream(t_items([shi], stages[G_HI]), t + 32, t + STEP + 32,
                       waits(wcopy(1, 1, 1), wcopy(1, 2, 0), wcopy(1, 2, 1)) if nc == 1 else None)
            add_units(leaf_units(l2get(0), stages[G_LO], slo, True, PR2_LOC[par], False,
                                 order=pure_first))
        units = leaf_units(l2get(1), stages[G_HI], shi, True, PR2_LOC[par], True, order=pure_first)
        t = now()
        if nc == 0:
            units = units[:28] + [(ge_unit, 1)] + units[28:]
        else:
            units = units[:28] + [fe_unit(nc - 1)] + units[28:]
        if nc + 1 < NCH:
            add_stream(t_items([slo + 2], stages[G_LO]), t + 32, t + sum(w for _, w in units) + 32,
                       waits(wcopy(1, 3, 0), wcopy(1, 3, 1), cp_wo) if nc == 2 else None)
        add_units(units)

    with _scope("main"):
        emit()

    with _scope("c2_tail"):
        for _, it in f_items(NCH - 1):
            it(None)
        fe_unit(NCH - 1)[0]()

    def ocopy(ch, r0, n, si):
        b, ck = ch // 4, ch % 4
        return pltpu.make_async_copy(
            obuf.at[ch, pl.ds(r0, n)],
            out_hbm.at[pl.ds((b * 250 + 64 * ck) * 8 + r0, n)], osems.at[si])

    ocps = []

    sub = jax.lax.broadcasted_iota(jnp.int32, (8, NL), 0)
    for ch in range(8):
      with _scope("joint%d" % ch):
        b, ck = ch // 4, ch % 4
        cols = []
        for lt in range(NCH):
            gev = ge[lt, pl.ds(16 * b, 8), :]
            god = ge[lt, pl.ds(16 * b + 8, 8), :]
            words = []
            for i in range(8):
                a2 = 8 * ck + i
                for k in range(1 if a2 == 31 else 4):
                    r0 = 2 * k * M + 2 * a2 + b
                    f0 = jnp.broadcast_to(fe[lt, r0:r0 + 1, :], (8, NL))
                    f1 = jnp.broadcast_to(fe[lt, r0 + M:r0 + M + 1, :], (8, NL))
                    ft = jnp.where(sub < 4, f0, f1)
                    words.append(pack2(jnp.tanh(ft + gev), jnp.tanh(ft + god)))
            cols.append(pltpu.bitcast(jnp.concatenate(words, axis=0), BF16))
        jv = jnp.concatenate(cols, axis=1)
        n = jv.shape[0]
        cuts = [0, n] if ch < 7 else [0, 128, 256, 384, n]
        for r0, r1 in zip(cuts[:-1], cuts[1:]):
            res = jnp.dot(jv[r0:r1], wo[...], preferred_element_type=F32)
            obuf[ch, r0:r1, :] = res.astype(BF16)
            ocps.append(ocopy(ch, r0, r1 - r0, len(ocps)))
            ocps[-1].start()
    for cp in ocps:
        cp.wait()


@jax.jit
def pallas_standalone__seq2seq_rnn_t_joint__speech_kernel(
    x: jax.Array,
    w1: jax.Array,
    w2: jax.Array,
    g: jax.Array,
    w_f: jax.Array,
    w_g: jax.Array,
    w_o: jax.Array,
):
    any_spec = pl.BlockSpec(memory_space=pl.ANY)
    out = pl.pallas_call(
        _kernel,
        out_shape=jax.ShapeDtypeStruct((B * 250 * NU, D), BF16),
        in_specs=[any_spec] * 7,
        out_specs=any_spec,
        scratch_shapes=[
            pltpu.VMEM((W_SUB, 256, NL), U32),
            pltpu.VMEM((54, 256, NL), U32),
            pltpu.VMEM((54, 256, NL), U32),
            pltpu.VMEM((54, 256, NL), U32),
            pltpu.VMEM((54, 192, NL), U32),
            pltpu.VMEM((54, 64, NL), U32),
            pltpu.VMEM((NSLOT_A, SR, NL), F32),
            pltpu.VMEM((81, 8, M // 2, NL), U32),
            pltpu.VMEM((B, T, D), BF16),
            pltpu.VMEM((B * NU, D), BF16),
            pltpu.VMEM((D, D), BF16),
            pltpu.VMEM((D, D), BF16),
            pltpu.VMEM((D, D), BF16),
            pltpu.VMEM((NCH, 512, NL), BF16),
            pltpu.VMEM((NCH, 512, NL), F32),
            pltpu.VMEM((NCH, 3 * B * NU, NL), F32),
            pltpu.VMEM((8, 512, D), BF16),
            pltpu.SMEM((1,), jnp.int32),
            pltpu.SemaphoreType.DMA((22,)),
            pltpu.SemaphoreType.DMA((11,)),
        ],
        compiler_params=pltpu.CompilerParams(vmem_limit_bytes=120 * 1024 * 1024),
    )(x, w1, w2, g.reshape(B * NU, D), w_f, w_g, w_o)
    return out.reshape(B, 250, NU, D)
```

```python
import jax
import jax.numpy as jnp
import jax.experimental.pallas as pl
import jax.experimental.pallas.tpu as pltpu

F32 = jnp.float32
BF16 = jnp.bfloat16
U32 = jnp.uint32

B, T, D, KT, NU = 2, 1000, 512, 31, 8
NL = 128
NCH = D // NL
M = 64
XP_ROWS = 1096
HB_BLK = 80
HB_ROWS = 16 * HB_BLK + 16
W_JUNK = 256
W_SUB = W_JUNK + 1
PR_ROWS = 27 * M
SR = 4384


class _Lazy:
    def __init__(self, fn):
        self.fn = fn
        self.v = None

    def get(self):
        if self.v is None:
            self.v = self.fn()
        return self.v


def _expand(vals, emit, base=0):
    n = len(vals)
    if n == 1:
        emit(base, vals[0])
        return
    h = n // 2
    third = 3 ** (h.bit_length() - 1)
    lo, hi = vals[:h], vals[h:]
    _expand(lo, emit, base)

    def add(a, b):
        return _Lazy(lambda: (a.get()[0] + b.get()[0], a.get()[1] + b.get()[1]))
    _expand([add(a, b) for a, b in zip(lo, hi)], emit, base + third)
    _expand(hi, emit, base + 2 * third)


def _pure_idx(k):
    if k == 0:
        return [0]
    sub = _pure_idx(k - 1)
    h = 2 ** (k - 1)
    return list(sub) + [None] * len(sub) + [None if i is None else i + h for i in sub]


PURE = _pure_idx(3)


def _in_expand(seq, n, emit, base=0):
    if n == 1:
        emit(base, seq[0])
        return
    h = n // 2
    third = 3 ** (h.bit_length() - 1)
    mid = seq[h:3 * h - 1]
    _in_expand([(a[0] - b[0], a[1] - b[1]) for a, b in zip(seq[0:2 * h - 1], mid)], h, emit, base)
    _in_expand(mid, h, emit, base + third)
    _in_expand([(a[0] - b[0], a[1] - b[1]) for a, b in zip(seq[2 * h:4 * h - 1], mid)], h, emit,
               base + 2 * third)


def _out_combine(get, base, n):
    if n == 1:
        return [get(base)]
    third = 3 ** ((n.bit_length() - 1) - 1)
    lo = _out_combine(get, base, n // 2)
    s = _out_combine(get, base + third, n // 2)
    out = [a + b for a, b in zip(s, lo)]
    hi = _out_combine(get, base + 2 * third, n // 2)
    out += [a + b for a, b in zip(s, hi)]
    return out


def _fold_slots(c):
    hi, low = c // 3 ** FOLD, c % 3 ** FOLD
    pats = [0]
    for i in range(FOLD):
        d = (low // 3 ** i) % 3
        bits = (0,) if d == 0 else ((0, 1) if d == 1 else (1,))
        pats = [p | (b << i) for p in pats for b in bits]
    return [hi * 2 ** FOLD + p for p in pats]


def _out_phases(get):
    nlow = 2 ** FOLD
    out = [None] * 8
    for rl in range(nlow):
        ys = _out_combine(lambda h: get(h * nlow + rl), 0, 8 // nlow)
        for rh, y in enumerate(ys):
            out[rh * nlow + rl] = y
    return out


def _gelu(x):
    c0 = 0.7978845608028654
    c1 = c0 * 0.044715
    inner = x * (c0 + c1 * (x * x))
    hx = 0.5 * x
    return hx + hx * jnp.tanh(inner)


class _Alloc:
    def __init__(self):
        self.fill = []

    def __call__(self, n):
        for s, f in enumerate(self.fill):
            if f + n <= SR:
                self.fill[s] += n
                return (s, f)
        self.fill.append(n)
        return (len(self.fill) - 1, 0)


_al = _Alloc()
XP_LOC = [_al(NCH * XP_ROWS) for _ in range(B)]
PR1_LOC = [[_al(PR_ROWS) for _ in range(3)] for _ in range(2)]
PR2_LOC = [_al(PR_ROWS) for _ in range(2)]
HB_LOC = [_al(HB_ROWS) for _ in range(NCH)]
JA_LOC = _al(64)
NSLOT_A = len(_al.fill)

G_LO, G_S, G_HI = 0, 1, 2

_PROFILE = False
FOLD = 1
TOKEN_LAG = 2


class _NoScope:
    def __enter__(self):
        return self

    def __exit__(self, *a):
        return False


def _scope(name):
    return jax.named_scope(name) if _PROFILE else _NoScope()


def _kernel(x_hbm, w1_hbm, w2_hbm, g_hbm, wf_hbm, wg_hbm, wo_hbm, out_hbm,
            aw, st0, st1, st2, l2a, l2b, aa, lhs1, xin, gin, wf, wg, wo,
            fbuf, fe, ge, obuf, zs, sems, osems):
    stages = [st0, st1, st2]
    aw16 = aw.bitcast(BF16)

    def wcopy(conv, nc, g):
        src = w1_hbm if conv == 0 else w2_hbm
        nt = 16 if g == 0 else 15
        slot = conv * 8 + nc * 2 + g
        return pltpu.make_async_copy(
            src.at[pl.ds(16 * g, nt), :, pl.ds(nc * NL, NL)],
            aw16.at[pl.ds(16 * slot, nt)], sems.at[slot])

    cp_x = [pltpu.make_async_copy(x_hbm.at[b], xin.at[b], sems.at[(16, 21)[b]]) for b in range(B)]
    cp_g = pltpu.make_async_copy(g_hbm, gin, sems.at[17])
    cp_wg = pltpu.make_async_copy(wg_hbm, wg, sems.at[18])
    cp_wf = pltpu.make_async_copy(wf_hbm, wf, sems.at[19])
    cp_wo = pltpu.make_async_copy(wo_hbm, wo, sems.at[20])

    for b in range(B):
        cp_x[b].start()
    for nc in range(NCH):
        for g in range(2):
            wcopy(0, nc, g).start()
    for nc in range(NCH):
        for g in range(2):
            wcopy(1, nc, g).start()
        if nc == 0:
            cp_g.start()
            cp_wg.start()
            cp_wf.start()
    cp_wo.start()

    for conv in range(2):
        for nc in range(NCH):
            aw[16 * (conv * 8 + nc * 2 + 1) + 15] = jnp.zeros((256, NL), U32)
    for b in range(B):
        s, o = XP_LOC[b]
        for lt in range(NCH):
            r0 = o + lt * XP_ROWS
            aa[s, r0:r0 + 16, :] = jnp.zeros((16, NL), F32)
            aa[s, r0 + 33 * 31 + 24:r0 + 33 * 33, :] = jnp.zeros((33 * 2 - 24, NL), F32)
    for lt in range(NCH):
        s, o = HB_LOC[lt]
        for blk in range(17):
            aa[s, o + blk * HB_BLK:o + blk * HB_BLK + 16, :] = jnp.zeros((16, NL), F32)

    zbox = []

    with _scope("p_xconv"):
        for b in range(B):
            cp_x[b].wait()
            s, o = XP_LOC[b]
            for lt in range(NCH):
                r0 = o + lt * XP_ROWS
                for gq in range(32):
                    t0, t1 = max(32 * gq - 16, 0), min(32 * gq + 16, T)
                    d0 = r0 + 33 * gq + (t0 - (32 * gq - 16))
                    aa[s, d0:d0 + (t1 - t0), :] = xin[b, t0:t1, lt * NL:(lt + 1) * NL].astype(F32)

    def pack2(a, b):
        return pltpu.pack_elementwise([a, b], packed_dtype=BF16).astype(U32)

    def lhs1_all():
        def body(i, carry):
            ag = i // 8
            kt = i % 8
            e = kt // 4
            lt = kt % 4
            base = lt * XP_ROWS + 33 * 8 * ag + e
            row = pl.multiple_of(ag * 8, 8)

            def ld(b, u):
                off = XP_LOC[b][1] + base + 2 * u + 1 + (1 if u >= 16 else 0)
                if u == 15:
                    off = off + e
                return aa[XP_LOC[b][0], pl.ds(off, 8, stride=33), :]

            for gi in (G_LO, G_HI, G_S):
                if gi == G_S:
                    seq = [tuple(ld(b, 8 + j) for b in range(B)) for j in range(15)]
                elif gi == G_LO:
                    seq = [tuple(ld(b, j) - ld(b, 8 + j) for b in range(B)) for j in range(15)]
                else:
                    seq = [tuple(ld(b, 16 + j) - ld(b, 8 + j) for b in range(B)) for j in range(15)]

                def put(c, v, gi=gi):
                    lhs1[gi * 27 + c, kt, pl.ds(row, 8), :] = pack2(v[0], v[1])
                _in_expand(seq, 8, put)
            zs[0] = i // 32
            return carry
        jax.lax.fori_loop(0, 32, body, 0)

    def unpack(v, h):
        return pltpu.unpack_elementwise(v, index=h, packed_dtype=BF16, unpacked_dtype=F32)

    def t_pos(slots, st, e, r):
        def fetch(m):
            raw = [aw[(zbox[0] if m == 0 else 0) + 16 * sl + 2 * m + e, pl.ds(r, 8), :] for sl in slots]
            if len(slots) == 2:
                return tuple(unpack(raw[0], h) + unpack(raw[1], h) for h in range(2))
            return tuple(unpack(raw[0], h) for h in range(2))
        src = [_Lazy(lambda m=m: fetch(m)) for m in range(8)]

        def put(c, v):
            if PURE[c] is None or len(slots) == 2:
                v = v.get()
                st[2 * c + e, pl.ds(r, 8), :] = pack2(v[0], v[1])
        _expand(src, put)
        last = 26 if len(slots) == 2 else 25
        return lambda: st[zbox[0] + 2 * last + e, pl.ds(r, 8), :]

    def fence(ref):
        def go(_):
            ref[zbox[0] + 54, 0:8, :] = jnp.zeros((8, NL), U32)
        return (None, go)

    def t_items(slots, st):
        return [(None, (lambda _, e=e, r=r: t_pos(slots, st, e, r)))
                for e in range(2) for r in range(0, 256, 8)] + [fence(st)]

    def d_items(nc):
        par = nc % 2
        hs, ho = HB_LOC[nc]

        def item(rb, k):
            sS, oS = PR1_LOC[par][G_S]
            sK, oK = PR1_LOC[par][G_LO if k == 0 else G_HI]

            def get(c):
                r = c * M + rb * 8
                return aa[(zbox[0] if c == 0 else 0) + sK, oK + r:oK + r + 8, :]
            ys = _out_phases(get)
            for r_ in range(8):
                p = 8 * k + r_
                y = _gelu(ys[r_])
                if rb == 7 and p >= 4:
                    rows = jax.lax.broadcasted_iota(jnp.int32, (8, NL), 0)
                    y = jnp.where(rows < 6, y, 0.0)
                r0 = ho + p * HB_BLK + 16 + rb * 8
                aa[hs, r0:r0 + 8, :] = y
        return [(None, (lambda _, rb=rb, k=k: item(rb, k))) for rb in range(8) for k in range(2)]

    def l2loc(kt):
        e, lt = kt // 4, kt % 4
        if lt == 3:
            return l2b, e * 32
        return l2a, (e * 3 + lt) * 32

    def e_items(nc):
        hs, ho = HB_LOC[nc]

        def item(j, e, ag, br):
            a0 = 8 * ag

            def ld(u):
                q = 2 * (8 * j + u) + e
                p = (q - 15) % 16
                c = (q - 15) // 16
                r0 = ho + p * HB_BLK + 16 + 2 * (a0 + c)
                return tuple(aa[(zbox[0] if u == 4 else 0) + hs, pl.ds(r0 + b, 8, stride=2), :] for b in range(B))

            def sub(a, b):
                return (a[0] - b[0], a[1] - b[1])
            mid = [ld(4 + i) for i in range(7)]
            if br == 1:
                seq = mid
            elif br == 0:
                seq = [sub(ld(i) if i < 4 else mid[i - 4], mid[i]) for i in range(7)]
            else:
                seq = [sub(ld(8 + i) if i >= 3 else mid[4 + i], mid[i]) for i in range(7)]
            l2, r0 = l2loc(e * 4 + nc)

            def put(c, v):
                l2[j * 27 + br * 9 + c, r0 + a0:r0 + a0 + 8, :] = pack2(v[0], v[1])
            _in_expand(seq, 4, put)
            return lambda: l2[zbox[0] + j * 27 + br * 9 + 8, r0 + a0:r0 + a0 + 8, :]
        return [(None, (lambda _, j=j, e=e, ag=ag, br=br: item(j, e, ag, br)))
                for j in range(2) for e in range(2) for ag in range(4) for br in range(3)
                ] + [fence(l2b if nc == 3 else l2a)]

    def f_items(nc):
        s2, o2 = PR2_LOC[nc % 2]

        def item(rb):
            def get(c):
                r = o2 + c * M + rb * 8
                return aa[(zbox[0] if c == 0 else 0) + s2, r:r + 8, :]
            ys = _out_phases(get)
            for p in range(8):
                fbuf[nc, p * M + rb * 8:p * M + rb * 8 + 8, :] = _gelu(ys[p]).astype(BF16)
        return [(None, (lambda _, rb=rb: item(rb))) for rb in range(8)]

    cnt = [0]

    no_pace_w = [False, 0]
    tokens = []

    def pace(v, wa=True):
        u = cnt[0] % 8
        cnt[0] += 1
        if not no_pace_w[0]:
            val = pltpu.bitcast(v, U32)
            while tokens and tokens[0][0] <= no_pace_w[1]:
                val = val ^ tokens.pop(0)[1]()
            aw[W_JUNK, 8 * u:8 * u + 8, :] = val
        if wa:
            aa[JA_LOC[0], JA_LOC[1] + 8 * u:JA_LOC[1] + 8 * u + 8, :] = v

    written = set()

    def leaf_units(lhs_get, st, slot, pure_ok, ploc, accumulate, order=None, lts=(0, 4),
                   into=None):
        units = []
        state = {}
        ps, po = ploc
        l0, l1 = lts

        def half(c, e):
            if pure_ok and PURE[c] is not None:
                w = aw[16 * slot + 2 * PURE[c] + e, 64 * l0:64 * l1, :]
            else:
                w = st[2 * c + e, 64 * l0:64 * l1, :]
            w = pltpu.bitcast(w, BF16)
            l = [pltpu.bitcast(lhs_get(c, e * 4 + k), BF16) for k in range(l0, l1)]
            l = jnp.concatenate(l, axis=1) if len(l) > 1 else l[0]
            return jnp.dot(l, w, preferred_element_type=F32)

        targets = into if into is not None else (ploc,)

        def commit(c, res):
            for loc in targets:
                for sl in _fold_slots(c):
                    rows = slice(loc[1] + sl * M, loc[1] + (sl + 1) * M)
                    if (loc, sl) in written:
                        aa[loc[0], rows, :] += res
                    else:
                        aa[loc[0], rows, :] = res
                        written.add((loc, sl))
            pace(res[M - 8:M], wa=False)

        def reset():
            for sl in range(27):
                written.discard((ploc, sl))

        first = [not accumulate and into is None]
        for c in (order if order is not None else range(27)):
            if l1 - l0 >= 2:
                def unit0(c=c):
                    if first[0]:
                        reset()
                        first[0] = False
                    res = half(c, 0)
                    state[c] = res
                    pace(res[M - 8:M])

                def unit1(c=c):
                    commit(c, half(c, 1) + state.pop(c))
                units += [(unit0, l1 - l0), (unit1, l1 - l0)]
            else:
                def unit01(c=c):
                    commit(c, half(c, 0) + half(c, 1))
                units.append((unit01, 2 * (l1 - l0)))
        return units

    tl_units = []
    tl_items = []

    def now():
        return float(sum(w for _, w in tl_units))

    def add_units(us):
        tl_units.extend(us)

    def add_stream(items, t0, t1, pre=None):
        n = len(items)
        for i, (ld, comp) in enumerate(items):
            tl_items.append((t0 + (i + 0.5) * (t1 - t0) / n, len(tl_items),
                             pre if i == 0 else None, ld, comp))

    def emit():
        seq = sorted(tl_items, key=lambda it: (it[0], it[1]))
        loaded = {}

        def preload(k):
            if k < len(seq) and k not in loaded:
                _, _, pre, ld, _ = seq[k]
                if pre is not None:
                    pre()
                loaded[k] = ld() if ld is not None else None

        ends = []
        t = 0.0
        for _, w in tl_units:
            t += w
            ends.append(t)
        quiet = set()
        for it in seq:
            if it[2] is not None:
                u = next(i for i, e in enumerate(ends) if it[0] < e)
                quiet.update((u, u - 1))
        k = 0
        for u, (fn, w) in enumerate(tl_units):
            no_pace_w[0] = u in quiet
            no_pace_w[1] = u
            fn()
            t = ends[u]
            while k < len(seq) and seq[k][0] < t:
                preload(k)
                if k + 1 < len(seq) and seq[k + 1][0] < t and seq[k + 1][2] is None:
                    preload(k + 1)
                tk = seq[k][4](loaded.pop(k))
                if tk is not None:
                    tokens.append((u + TOKEN_LAG, tk))
                k += 1
        no_pace_w[0] = False
        assert k == len(seq)

    with _scope("p_lhs1"):
        lhs1_all()
    zbox.append(zs[0])

    def l1get(gi):
        return lambda c, kt: lhs1[gi * 27 + c, kt]

    def l2get(j):
        def get(c, kt):
            l2, r0 = l2loc(kt)
            return l2[j * 27 + c, r0:r0 + 32, :]
        return get

    def fe_unit(kc):
        def unit():
            res = jnp.dot(fbuf[kc], wf[kc * NL:(kc + 1) * NL, :], preferred_element_type=F32)
            for lt in range(NCH):
                if kc == 0:
                    fe[lt] = res[:, lt * NL:(lt + 1) * NL]
                else:
                    fe[lt] += res[:, lt * NL:(lt + 1) * NL]
        return (unit, 32)

    def waits(*cps):
        def go():
            for cp in cps:
                cp.wait()
        return go

    def ge_unit():
        res = jnp.dot(gin[...], wg[...], preferred_element_type=F32)
        for lt in range(NCH):
            ge[lt, 32:48, :] = res[:, lt * NL:(lt + 1) * NL]
        for lt in range(NCH):
            for b in range(B):
                for par in range(2):
                    v = ge[lt, pl.ds(32 + 8 * b + par, 4, stride=2), :]
                    ge[lt, 16 * b + 8 * par:16 * b + 8 * par + 4, :] = v
                    ge[lt, 16 * b + 8 * par + 4:16 * b + 8 * par + 8, :] = v

    pure_first = ([c for c in range(27) if PURE[c] is not None]
                  + [c for c in range(27) if PURE[c] is None])
    STEP = 54 * 4.0

    wcopy(0, 0, 0).wait()
    for nc in range(NCH):
        par = nc % 2
        slo, shi = nc * 2, nc * 2 + 1
        t = now()
        if nc == 0:
            add_stream(t_items([slo], stages[G_LO]), t, t + 60)
            add_stream(t_items([shi], stages[G_HI]), t + 140, t + STEP + 56, wcopy(0, nc, 1).wait)
            add_stream(t_items([slo, shi], stages[G_S]), t + STEP + 56, t + 2 * STEP - 12)
        else:
            add_stream(t_items([shi], stages[G_HI]), t - 44, t + 139,
                       wcopy(0, nc, 1).wait if nc < 2 else None)
            add_stream(t_items([slo, shi], stages[G_S]), t + 139, t + 2 * STEP - 12)
            add_stream(d_items(nc - 1), t, t + 330)
            add_stream(e_items(nc - 1), t + 330, t + 3 * STEP - 44)
        if nc + 1 < NCH:
            add_stream(t_items([slo + 2], stages[G_LO]), t + 2 * STEP - 12, t + 3 * STEP - 44,
                       wcopy(0, nc + 1, 0).wait if nc < 1 else
                       waits(wcopy(0, nc + 1, 0), wcopy(0, nc + 1, 1)))
        else:
            add_stream(t_items([8], stages[G_LO]), t + 2 * STEP - 12, t + 3 * STEP,
                       waits(cp_g, cp_wg, cp_wf, wcopy(1, 0, 0), wcopy(1, 0, 1)))
        add_units(leaf_units(l1get(G_LO), stages[G_LO], slo, True, PR1_LOC[par][G_LO], False,
                             order=pure_first))
        add_units(leaf_units(l1get(G_HI), stages[G_HI], shi, True, PR1_LOC[par][G_HI], False,
                             order=pure_first))
        add_units(leaf_units(l1get(G_S), stages[G_S], None, False, PR1_LOC[par][G_S], False,
                             into=(PR1_LOC[par][G_LO], PR1_LOC[par][G_HI])))

    for nc in range(NCH):
        par = nc % 2
        slo, shi = 8 + nc * 2, 8 + nc * 2 + 1
        t = now()
        if nc == 0:
            add_stream(d_items(NCH - 1), t, t + 0.3 * STEP)
            add_stream(e_items(NCH - 1), t + 0.3 * STEP, t + 0.72 * STEP)
            add_stream(t_items([shi], stages[G_HI]), t, t + STEP + 32)
            add_units(leaf_units(l2get(0), stages[G_LO], slo, True, PR2_LOC[par], False, lts=(0, 3),
                                 order=pure_first))
            add_units(leaf_units(l2get(0), stages[G_LO], slo, True, PR2_LOC[par], True, lts=(3, 4)))
        else:
            add_stream(f_items(nc - 1), t, t + STEP)
            add_stream(t_items([shi], stages[G_HI]), t + 32, t + STEP + 32)
            add_units(leaf_units(l2get(0), stages[G_LO], slo, True, PR2_LOC[par], False,
                                 order=pure_first))
        units = leaf_units(l2get(1), stages[G_HI], shi, True, PR2_LOC[par], True, order=pure_first)
        t = now()
        if nc == 0:
            units = units[:28] + [(ge_unit, 1)] + units[28:]
        else:
            units = units[:28] + [fe_unit(nc - 1)] + units[28:]
        if nc + 1 < NCH:
            add_stream(t_items([slo + 2], stages[G_LO]), t + 32, t + sum(w for _, w in units) + 32,
                       waits(wcopy(1, nc + 1, 0), wcopy(1, nc + 1, 1)))
        add_units(units)

    with _scope("main"):
        emit()

    with _scope("c2_tail"):
        for _, it in f_items(NCH - 1):
            it(None)
        fe_unit(NCH - 1)[0]()

    cp_wo.wait()

    def ocopy(ch, r0, n, si):
        b, ck = ch // 4, ch % 4
        return pltpu.make_async_copy(
            obuf.at[ch, pl.ds(r0, n)],
            out_hbm.at[pl.ds((b * 250 + 64 * ck) * 8 + r0, n)], osems.at[si])

    ocps = []

    sub = jax.lax.broadcasted_iota(jnp.int32, (8, NL), 0)
    for ch in range(8):
      with _scope("joint%d" % ch):
        b, ck = ch // 4, ch % 4
        cols = []
        for lt in range(NCH):
            gev = ge[lt, pl.ds(16 * b, 8), :]
            god = ge[lt, pl.ds(16 * b + 8, 8), :]
            words = []
            for i in range(8):
                a2 = 8 * ck + i
                for k in range(1 if a2 == 31 else 4):
                    r0 = 2 * k * M + 2 * a2 + b
                    f0 = jnp.broadcast_to(fe[lt, r0:r0 + 1, :], (8, NL))
                    f1 = jnp.broadcast_to(fe[lt, r0 + M:r0 + M + 1, :], (8, NL))
                    ft = jnp.where(sub < 4, f0, f1)
                    words.append(pack2(jnp.tanh(ft + gev), jnp.tanh(ft + god)))
            cols.append(pltpu.bitcast(jnp.concatenate(words, axis=0), BF16))
        jv = jnp.concatenate(cols, axis=1)
        n = jv.shape[0]
        cuts = [0, n] if ch < 7 else [0, 128, 256, 384, n]
        for r0, r1 in zip(cuts[:-1], cuts[1:]):
            res = jnp.dot(jv[r0:r1], wo[...], preferred_element_type=F32)
            obuf[ch, r0:r1, :] = res.astype(BF16)
            ocps.append(ocopy(ch, r0, r1 - r0, len(ocps)))
            ocps[-1].start()
    for cp in ocps:
        cp.wait()


@jax.jit
def pallas_standalone__seq2seq_rnn_t_joint__speech_kernel(
    x: jax.Array,
    w1: jax.Array,
    w2: jax.Array,
    g: jax.Array,
    w_f: jax.Array,
    w_g: jax.Array,
    w_o: jax.Array,
):
    any_spec = pl.BlockSpec(memory_space=pl.ANY)
    out = pl.pallas_call(
        _kernel,
        out_shape=jax.ShapeDtypeStruct((B * 250 * NU, D), BF16),
        in_specs=[any_spec] * 7,
        out_specs=any_spec,
        scratch_shapes=[
            pltpu.VMEM((W_SUB, 256, NL), U32),
            pltpu.VMEM((55, 256, NL), U32),
            pltpu.VMEM((55, 256, NL), U32),
            pltpu.VMEM((55, 256, NL), U32),
            pltpu.VMEM((55, 192, NL), U32),
            pltpu.VMEM((55, 64, NL), U32),
            pltpu.VMEM((NSLOT_A, SR, NL), F32),
            pltpu.VMEM((81, 8, M // 2, NL), U32),
            pltpu.VMEM((B, T, D), BF16),
            pltpu.VMEM((B * NU, D), BF16),
            pltpu.VMEM((D, D), BF16),
            pltpu.VMEM((D, D), BF16),
            pltpu.VMEM((D, D), BF16),
            pltpu.VMEM((NCH, 512, NL), BF16),
            pltpu.VMEM((NCH, 512, NL), F32),
            pltpu.VMEM((NCH, 3 * B * NU, NL), F32),
            pltpu.VMEM((8, 512, D), BF16),
            pltpu.SMEM((1,), jnp.int32),
            pltpu.SemaphoreType.DMA((22,)),
            pltpu.SemaphoreType.DMA((11,)),
        ],
        compiler_params=pltpu.CompilerParams(vmem_limit_bytes=120 * 1024 * 1024),
    )(x, w1, w2, g.reshape(B * NU, D), w_f, w_g, w_o)
    return out.reshape(B, 250, NU, D)
```

```python
import jax
import jax.numpy as jnp
import jax.experimental.pallas as pl
import jax.experimental.pallas.tpu as pltpu

F32 = jnp.float32
BF16 = jnp.bfloat16
U32 = jnp.uint32

B, T, D, KT, NU = 2, 1000, 512, 31, 8
NL = 128
NCH = D // NL
M = 64
XP_ROWS = 1096
HB_BLK = 80
HB_ROWS = 16 * HB_BLK + 16
W_JUNK = 256
W_SUB = W_JUNK + 1
PR_ROWS = 27 * M
SR = 4384


class _Lazy:
    def __init__(self, fn):
        self.fn = fn
        self.v = None

    def get(self):
        if self.v is None:
            self.v = self.fn()
        return self.v


def _expand(vals, emit, base=0):
    n = len(vals)
    if n == 1:
        emit(base, vals[0])
        return
    h = n // 2
    third = 3 ** (h.bit_length() - 1)
    lo, hi = vals[:h], vals[h:]
    _expand(lo, emit, base)

    def add(a, b):
        return _Lazy(lambda: (a.get()[0] + b.get()[0], a.get()[1] + b.get()[1]))
    _expand([add(a, b) for a, b in zip(lo, hi)], emit, base + third)
    _expand(hi, emit, base + 2 * third)


def _pure_idx(k):
    if k == 0:
        return [0]
    sub = _pure_idx(k - 1)
    h = 2 ** (k - 1)
    return list(sub) + [None] * len(sub) + [None if i is None else i + h for i in sub]


PURE = _pure_idx(3)


def _in_expand(seq, n, emit, base=0):
    if n == 1:
        emit(base, seq[0])
        return
    h = n // 2
    third = 3 ** (h.bit_length() - 1)
    mid = seq[h:3 * h - 1]
    _in_expand([(a[0] - b[0], a[1] - b[1]) for a, b in zip(seq[0:2 * h - 1], mid)], h, emit, base)
    _in_expand(mid, h, emit, base + third)
    _in_expand([(a[0] - b[0], a[1] - b[1]) for a, b in zip(seq[2 * h:4 * h - 1], mid)], h, emit,
               base + 2 * third)


def _out_combine(get, base, n):
    if n == 1:
        return [get(base)]
    third = 3 ** ((n.bit_length() - 1) - 1)
    lo = _out_combine(get, base, n // 2)
    s = _out_combine(get, base + third, n // 2)
    out = [a + b for a, b in zip(s, lo)]
    hi = _out_combine(get, base + 2 * third, n // 2)
    out += [a + b for a, b in zip(s, hi)]
    return out


def _fold_slots(c):
    hi, low = c // 3 ** FOLD, c % 3 ** FOLD
    pats = [0]
    for i in range(FOLD):
        d = (low // 3 ** i) % 3
        bits = (0,) if d == 0 else ((0, 1) if d == 1 else (1,))
        pats = [p | (b << i) for p in pats for b in bits]
    return [hi * 2 ** FOLD + p for p in pats]


def _out_phases(get):
    nlow = 2 ** FOLD
    out = [None] * 8
    for rl in range(nlow):
        ys = _out_combine(lambda h: get(h * nlow + rl), 0, 8 // nlow)
        for rh, y in enumerate(ys):
            out[rh * nlow + rl] = y
    return out


def _gelu(x):
    c0 = 0.7978845608028654
    c1 = c0 * 0.044715
    inner = x * (c0 + c1 * (x * x))
    hx = 0.5 * x
    return hx + hx * jnp.tanh(inner)


class _Alloc:
    def __init__(self):
        self.fill = []

    def __call__(self, n):
        for s, f in enumerate(self.fill):
            if f + n <= SR:
                self.fill[s] += n
                return (s, f)
        self.fill.append(n)
        return (len(self.fill) - 1, 0)


_al = _Alloc()
XP_LOC = [_al(NCH * XP_ROWS) for _ in range(B)]
PR1_LOC = [[_al(PR_ROWS) for _ in range(3)] for _ in range(2)]
PR2_LOC = [_al(PR_ROWS) for _ in range(2)]
HB_LOC = [_al(HB_ROWS) for _ in range(NCH)]
JA_LOC = _al(64)
NSLOT_A = len(_al.fill)

G_LO, G_S, G_HI = 0, 1, 2

_PROFILE = False
FOLD = 1
TOKEN_LAG = 2


class _NoScope:
    def __enter__(self):
        return self

    def __exit__(self, *a):
        return False


def _scope(name):
    return jax.named_scope(name) if _PROFILE else _NoScope()


def _kernel(x_hbm, w1_hbm, w2_hbm, g_hbm, wf_hbm, wg_hbm, wo_hbm, out_hbm,
            aw, st0, st1, st2, l2a, l2b, aa, lhs1, xin, gin, wf, wg, wo,
            fbuf, fe, ge, obuf, zs, sems, osems):
    stages = [st0, st1, st2]
    aw16 = aw.bitcast(BF16)

    def wcopy(conv, nc, g):
        src = w1_hbm if conv == 0 else w2_hbm
        nt = 16 if g == 0 else 15
        slot = conv * 8 + nc * 2 + g
        return pltpu.make_async_copy(
            src.at[pl.ds(16 * g, nt), :, pl.ds(nc * NL, NL)],
            aw16.at[pl.ds(16 * slot, nt)], sems.at[slot])

    cp_x = [pltpu.make_async_copy(x_hbm.at[b], xin.at[b], sems.at[(16, 21)[b]]) for b in range(B)]
    cp_g = pltpu.make_async_copy(g_hbm, gin, sems.at[17])
    cp_wg = pltpu.make_async_copy(wg_hbm, wg, sems.at[18])
    cp_wf = pltpu.make_async_copy(wf_hbm, wf, sems.at[19])
    cp_wo = pltpu.make_async_copy(wo_hbm, wo, sems.at[20])

    for b in range(B):
        cp_x[b].start()
    for nc in range(NCH):
        for g in range(2):
            wcopy(0, nc, g).start()
    for nc in range(NCH):
        for g in range(2):
            wcopy(1, nc, g).start()
        if nc == 0:
            cp_g.start()
            cp_wg.start()
            cp_wf.start()
    cp_wo.start()

    for conv in range(2):
        for nc in range(NCH):
            aw[16 * (conv * 8 + nc * 2 + 1) + 15] = jnp.zeros((256, NL), U32)
    for b in range(B):
        s, o = XP_LOC[b]
        for lt in range(NCH):
            r0 = o + lt * XP_ROWS
            aa[s, r0:r0 + 16, :] = jnp.zeros((16, NL), F32)
            aa[s, r0 + 33 * 31 + 24:r0 + 33 * 33, :] = jnp.zeros((33 * 2 - 24, NL), F32)
    for lt in range(NCH):
        s, o = HB_LOC[lt]
        for blk in range(17):
            aa[s, o + blk * HB_BLK:o + blk * HB_BLK + 16, :] = jnp.zeros((16, NL), F32)

    zbox = []

    with _scope("p_xconv"):
        for b in range(B):
            cp_x[b].wait()
            s, o = XP_LOC[b]
            for lt in range(NCH):
                r0 = o + lt * XP_ROWS
                for gq in range(32):
                    t0, t1 = max(32 * gq - 16, 0), min(32 * gq + 16, T)
                    d0 = r0 + 33 * gq + (t0 - (32 * gq - 16))
                    aa[s, d0:d0 + (t1 - t0), :] = xin[b, t0:t1, lt * NL:(lt + 1) * NL].astype(F32)

    def pack2(a, b):
        return pltpu.pack_elementwise([a, b], packed_dtype=BF16).astype(U32)

    def lhs1_all():
        def body(i, carry):
            ag = jax.lax.shift_right_logical(i, 3)
            kt = i & 7
            e = jax.lax.shift_right_logical(kt, 2)
            lt = kt & 3
            base = lt * XP_ROWS + 33 * 8 * ag + e
            row = pl.multiple_of(ag * 8, 8)

            def ld(b, u):
                off = XP_LOC[b][1] + base + 2 * u + 1 + (1 if u >= 16 else 0)
                if u == 15:
                    off = off + e
                return aa[XP_LOC[b][0], pl.ds(off, 8, stride=33), :]

            for gi in (G_LO, G_HI, G_S):
                if gi == G_S:
                    seq = [tuple(ld(b, 8 + j) for b in range(B)) for j in range(15)]
                elif gi == G_LO:
                    seq = [tuple(ld(b, j) - ld(b, 8 + j) for b in range(B)) for j in range(15)]
                else:
                    seq = [tuple(ld(b, 16 + j) - ld(b, 8 + j) for b in range(B)) for j in range(15)]

                def put(c, v, gi=gi):
                    lhs1[gi * 27 + c, kt, pl.ds(row, 8), :] = pack2(v[0], v[1])
                _in_expand(seq, 8, put)
            zs[0] = jax.lax.shift_right_logical(i, 5)
            return carry
        jax.lax.fori_loop(0, 32, body, 0)

    def unpack(v, h):
        return pltpu.unpack_elementwise(v, index=h, packed_dtype=BF16, unpacked_dtype=F32)

    def t_pos(slots, st, e, r):
        def fetch(m):
            raw = [aw[(zbox[0] if m == 0 else 0) + 16 * sl + 2 * m + e, pl.ds(r, 8), :] for sl in slots]
            if len(slots) == 2:
                return tuple(unpack(raw[0], h) + unpack(raw[1], h) for h in range(2))
            return tuple(unpack(raw[0], h) for h in range(2))
        src = [_Lazy(lambda m=m: fetch(m)) for m in range(8)]

        def put(c, v):
            if PURE[c] is None or len(slots) == 2:
                v = v.get()
                st[2 * c + e, pl.ds(r, 8), :] = pack2(v[0], v[1])
        _expand(src, put)
        last = 26 if len(slots) == 2 else 25
        return lambda: st[zbox[0] + 2 * last + e, pl.ds(r, 8), :]

    def fence(ref):
        def go(_):
            ref[zbox[0] + 54, 0:8, :] = jnp.zeros((8, NL), U32)
        return (None, go)

    def t_items(slots, st):
        return [(None, (lambda _, e=e, r=r: t_pos(slots, st, e, r)))
                for e in range(2) for r in range(0, 256, 8)] + [fence(st)]

    def d_items(nc):
        par = nc % 2
        hs, ho = HB_LOC[nc]

        def item(rb, k):
            sK, oK = PR1_LOC[par][G_LO if k == 0 else G_HI]

            def get(c):
                r = c * M + rb * 8
                return aa[(zbox[0] if c == 0 else 0) + sK, oK + r:oK + r + 8, :]
            ys = _out_phases(get)
            for r_ in range(8):
                p = 8 * k + r_
                y = _gelu(ys[r_])
                if rb == 7 and p >= 4:
                    rows = jax.lax.broadcasted_iota(jnp.int32, (8, NL), 0)
                    y = jnp.where(rows < 6, y, 0.0)
                r0 = ho + p * HB_BLK + 16 + rb * 8
                aa[hs, r0:r0 + 8, :] = y
        return [(None, (lambda _, rb=rb, k=k: item(rb, k))) for rb in range(8) for k in range(2)]

    def l2loc(kt):
        e, lt = kt // 4, kt % 4
        if lt == 3:
            return l2b, e * 32
        return l2a, (e * 3 + lt) * 32

    def e_items(nc):
        hs, ho = HB_LOC[nc]

        def item(j, e, ag, br):
            a0 = 8 * ag

            def ld(u):
                q = 2 * (8 * j + u) + e
                p = (q - 15) % 16
                c = (q - 15) // 16
                r0 = ho + p * HB_BLK + 16 + 2 * (a0 + c)
                return tuple(aa[(zbox[0] if u == 4 else 0) + hs, pl.ds(r0 + b, 8, stride=2), :] for b in range(B))

            def sub(a, b):
                return (a[0] - b[0], a[1] - b[1])
            mid = [ld(4 + i) for i in range(7)]
            if br == 1:
                seq = mid
            elif br == 0:
                seq = [sub(ld(i) if i < 4 else mid[i - 4], mid[i]) for i in range(7)]
            else:
                seq = [sub(ld(8 + i) if i >= 3 else mid[4 + i], mid[i]) for i in range(7)]
            l2, r0 = l2loc(e * 4 + nc)

            def put(c, v):
                l2[j * 27 + br * 9 + c, r0 + a0:r0 + a0 + 8, :] = pack2(v[0], v[1])
            _in_expand(seq, 4, put)
            return lambda: l2[zbox[0] + j * 27 + br * 9 + 8, r0 + a0:r0 + a0 + 8, :]
        return [(None, (lambda _, j=j, e=e, ag=ag, br=br: item(j, e, ag, br)))
                for j in range(2) for e in range(2) for ag in range(4) for br in range(3)
                ] + [fence(l2b if nc == 3 else l2a)]

    def f_items(nc):
        s2, o2 = PR2_LOC[nc % 2]

        def item(rb):
            def get(c):
                r = o2 + c * M + rb * 8
                return aa[(zbox[0] if c == 0 else 0) + s2, r:r + 8, :]
            ys = _out_phases(get)
            for p in range(8):
                fbuf[nc, p * M + rb * 8:p * M + rb * 8 + 8, :] = _gelu(ys[p]).astype(BF16)
        return [(None, (lambda _, rb=rb: item(rb))) for rb in range(8)]

    cnt = [0]

    no_pace_w = [False, 0]
    tokens = []

    def pace(v, wa=True):
        u = cnt[0] % 8
        cnt[0] += 1
        if not no_pace_w[0]:
            val = pltpu.bitcast(v, U32)
            while tokens and tokens[0][0] <= no_pace_w[1]:
                val = val ^ tokens.pop(0)[1]()
            aw[W_JUNK, 8 * u:8 * u + 8, :] = val
        if wa:
            aa[JA_LOC[0], JA_LOC[1] + 8 * u:JA_LOC[1] + 8 * u + 8, :] = v

    written = set()

    def leaf_units(lhs_get, st, slot, pure_ok, ploc, accumulate, order=None, lts=(0, 4),
                   into=None):
        units = []
        state = {}
        ps, po = ploc
        l0, l1 = lts

        def half(c, e):
            if pure_ok and PURE[c] is not None:
                w = aw[16 * slot + 2 * PURE[c] + e, 64 * l0:64 * l1, :]
            else:
                w = st[2 * c + e, 64 * l0:64 * l1, :]
            w = pltpu.bitcast(w, BF16)
            l = [pltpu.bitcast(lhs_get(c, e * 4 + k), BF16) for k in range(l0, l1)]
            l = jnp.concatenate(l, axis=1) if len(l) > 1 else l[0]
            return jnp.dot(l, w, preferred_element_type=F32)

        targets = into if into is not None else (ploc,)

        def commit(c, res):
            for loc in targets:
                for sl in _fold_slots(c):
                    rows = slice(loc[1] + sl * M, loc[1] + (sl + 1) * M)
                    if (loc, sl) in written:
                        aa[loc[0], rows, :] += res
                    else:
                        aa[loc[0], rows, :] = res
                        written.add((loc, sl))
            pace(res[M - 8:M], wa=False)

        def reset():
            for sl in range(27):
                written.discard((ploc, sl))

        first = [not accumulate and into is None]
        for c in (order if order is not None else range(27)):
            if l1 - l0 >= 2:
                def unit0(c=c):
                    if first[0]:
                        reset()
                        first[0] = False
                    res = half(c, 0)
                    state[c] = res
                    pace(res[M - 8:M])

                def unit1(c=c):
                    commit(c, half(c, 1) + state.pop(c))
                units += [(unit0, l1 - l0), (unit1, l1 - l0)]
            else:
                def unit01(c=c):
                    commit(c, half(c, 0) + half(c, 1))
                units.append((unit01, 2 * (l1 - l0)))
        return units

    tl_units = []
    tl_items = []

    def now():
        return float(sum(w for _, w in tl_units))

    def add_units(us):
        tl_units.extend(us)

    def add_stream(items, t0, t1, pre=None):
        n = len(items)
        for i, (ld, comp) in enumerate(items):
            tl_items.append((t0 + (i + 0.5) * (t1 - t0) / n, len(tl_items),
                             pre if i == 0 else None, ld, comp))

    def emit():
        seq = sorted(tl_items, key=lambda it: (it[0], it[1]))
        loaded = {}

        def preload(k):
            if k < len(seq) and k not in loaded:
                _, _, pre, ld, _ = seq[k]
                if pre is not None:
                    pre()
                loaded[k] = ld() if ld is not None else None

        ends = []
        t = 0.0
        for _, w in tl_units:
            t += w
            ends.append(t)
        quiet = set()
        for it in seq:
            if it[2] is not None:
                u = next(i for i, e in enumerate(ends) if it[0] < e)
                quiet.update((u, u - 1))
        k = 0
        for u, (fn, w) in enumerate(tl_units):
            no_pace_w[0] = u in quiet
            no_pace_w[1] = u
            fn()
            t = ends[u]
            while k < len(seq) and seq[k][0] < t:
                preload(k)
                if k + 1 < len(seq) and seq[k + 1][0] < t and seq[k + 1][2] is None:
                    preload(k + 1)
                tk = seq[k][4](loaded.pop(k))
                if tk is not None:
                    tokens.append((u + TOKEN_LAG, tk))
                k += 1
        no_pace_w[0] = False
        assert k == len(seq)

    with _scope("p_lhs1"):
        lhs1_all()
    zbox.append(zs[0])

    def l1get(gi):
        return lambda c, kt: lhs1[gi * 27 + c, kt]

    def l2get(j):
        def get(c, kt):
            l2, r0 = l2loc(kt)
            return l2[j * 27 + c, r0:r0 + 32, :]
        return get

    def fe_unit(kc):
        def unit():
            res = jnp.dot(fbuf[kc], wf[kc * NL:(kc + 1) * NL, :], preferred_element_type=F32)
            for lt in range(NCH):
                if kc == 0:
                    fe[lt] = res[:, lt * NL:(lt + 1) * NL]
                else:
                    fe[lt] += res[:, lt * NL:(lt + 1) * NL]
        return (unit, 32)

    def waits(*cps):
        def go():
            for cp in cps:
                cp.wait()
        return go

    def ge_unit():
        res = jnp.dot(gin[...], wg[...], preferred_element_type=F32)
        for lt in range(NCH):
            ge[lt, 32:48, :] = res[:, lt * NL:(lt + 1) * NL]
        for lt in range(NCH):
            for b in range(B):
                for par in range(2):
                    v = ge[lt, pl.ds(32 + 8 * b + par, 4, stride=2), :]
                    ge[lt, 16 * b + 8 * par:16 * b + 8 * par + 4, :] = v
                    ge[lt, 16 * b + 8 * par + 4:16 * b + 8 * par + 8, :] = v

    pure_first = ([c for c in range(27) if PURE[c] is not None]
                  + [c for c in range(27) if PURE[c] is None])
    STEP = 54 * 4.0

    wcopy(0, 0, 0).wait()
    for nc in range(NCH):
        par = nc % 2
        slo, shi = nc * 2, nc * 2 + 1
        t = now()
        if nc == 0:
            add_stream(t_items([slo], stages[G_LO]), t, t + 60)
            add_stream(t_items([shi], stages[G_HI]), t + 140, t + STEP + 56, wcopy(0, nc, 1).wait)
            add_stream(t_items([slo, shi], stages[G_S]), t + STEP + 56, t + 2 * STEP - 12)
        else:
            add_stream(t_items([shi], stages[G_HI]), t - 44, t + 139,
                       wcopy(0, nc, 1).wait if nc < 2 else None)
            add_stream(t_items([slo, shi], stages[G_S]), t + 139, t + 2 * STEP - 12)
            add_stream(d_items(nc - 1), t, t + 330)
            add_stream(e_items(nc - 1), t + 330, t + 3 * STEP - 44)
        if nc + 1 < NCH:
            add_stream(t_items([slo + 2], stages[G_LO]), t + 2 * STEP - 12, t + 3 * STEP - 44,
                       wcopy(0, nc + 1, 0).wait if nc < 1 else
                       waits(wcopy(0, nc + 1, 0), wcopy(0, nc + 1, 1)))
        else:
            add_stream(t_items([8], stages[G_LO]), t + 2 * STEP - 12, t + 3 * STEP,
                       waits(cp_g, cp_wg, cp_wf, wcopy(1, 0, 0), wcopy(1, 0, 1)))
        add_units(leaf_units(l1get(G_LO), stages[G_LO], slo, True, PR1_LOC[par][G_LO], False,
                             order=pure_first))
        add_units(leaf_units(l1get(G_HI), stages[G_HI], shi, True, PR1_LOC[par][G_HI], False,
                             order=pure_first))
        add_units(leaf_units(l1get(G_S), stages[G_S], None, False, PR1_LOC[par][G_S], False,
                             into=(PR1_LOC[par][G_LO], PR1_LOC[par][G_HI])))

    for nc in range(NCH):
        par = nc % 2
        slo, shi = 8 + nc * 2, 8 + nc * 2 + 1
        t = now()
        if nc == 0:
            add_stream(d_items(NCH - 1), t, t + 0.3 * STEP)
            add_stream(e_items(NCH - 1), t + 0.3 * STEP, t + 0.72 * STEP)
            add_stream(t_items([shi], stages[G_HI]), t, t + STEP + 32)
            add_units(leaf_units(l2get(0), stages[G_LO], slo, True, PR2_LOC[par], False, lts=(0, 3),
                                 order=pure_first))
            add_units(leaf_units(l2get(0), stages[G_LO], slo, True, PR2_LOC[par], True, lts=(3, 4)))
        else:
            add_stream(f_items(nc - 1), t, t + STEP)
            add_stream(t_items([shi], stages[G_HI]), t + 32, t + STEP + 32)
            add_units(leaf_units(l2get(0), stages[G_LO], slo, True, PR2_LOC[par], False,
                                 order=pure_first))
        units = leaf_units(l2get(1), stages[G_HI], shi, True, PR2_LOC[par], True, order=pure_first)
        t = now()
        if nc == 0:
            units = units[:28] + [(ge_unit, 1)] + units[28:]
        else:
            units = units[:28] + [fe_unit(nc - 1)] + units[28:]
        if nc + 1 < NCH:
            add_stream(t_items([slo + 2], stages[G_LO]), t + 32, t + sum(w for _, w in units) + 32,
                       waits(wcopy(1, nc + 1, 0), wcopy(1, nc + 1, 1)))
        add_units(units)

    with _scope("main"):
        emit()

    with _scope("c2_tail"):
        for _, it in f_items(NCH - 1):
            it(None)
        fe_unit(NCH - 1)[0]()

    cp_wo.wait()

    def ocopy(ch, r0, n, si):
        b, ck = ch // 4, ch % 4
        return pltpu.make_async_copy(
            obuf.at[ch, pl.ds(r0, n)],
            out_hbm.at[pl.ds((b * 250 + 64 * ck) * 8 + r0, n)], osems.at[si])

    ocps = []

    sub = jax.lax.broadcasted_iota(jnp.int32, (8, NL), 0)
    for ch in range(8):
      with _scope("joint%d" % ch):
        b, ck = ch // 4, ch % 4
        cols = []
        for lt in range(NCH):
            gev = ge[lt, pl.ds(16 * b, 8), :]
            god = ge[lt, pl.ds(16 * b + 8, 8), :]
            words = []
            for i in range(8):
                a2 = 8 * ck + i
                for k in range(1 if a2 == 31 else 4):
                    r0 = 2 * k * M + 2 * a2 + b
                    f0 = jnp.broadcast_to(fe[lt, r0:r0 + 1, :], (8, NL))
                    f1 = jnp.broadcast_to(fe[lt, r0 + M:r0 + M + 1, :], (8, NL))
                    ft = jnp.where(sub < 4, f0, f1)
                    words.append(pack2(jnp.tanh(ft + gev), jnp.tanh(ft + god)))
            cols.append(pltpu.bitcast(jnp.concatenate(words, axis=0), BF16))
        jv = jnp.concatenate(cols, axis=1)
        n = jv.shape[0]
        cuts = [0, n] if ch < 7 else [0, 128, 256, 384, n]
        for r0, r1 in zip(cuts[:-1], cuts[1:]):
            res = jnp.dot(jv[r0:r1], wo[...], preferred_element_type=F32)
            obuf[ch, r0:r1, :] = res.astype(BF16)
            ocps.append(ocopy(ch, r0, r1 - r0, len(ocps)))
            ocps[-1].start()
    for cp in ocps:
        cp.wait()


@jax.jit
def pallas_standalone__seq2seq_rnn_t_joint__speech_kernel(
    x: jax.Array,
    w1: jax.Array,
    w2: jax.Array,
    g: jax.Array,
    w_f: jax.Array,
    w_g: jax.Array,
    w_o: jax.Array,
):
    any_spec = pl.BlockSpec(memory_space=pl.ANY)
    out = pl.pallas_call(
        _kernel,
        out_shape=jax.ShapeDtypeStruct((B * 250 * NU, D), BF16),
        in_specs=[any_spec] * 7,
        out_specs=any_spec,
        scratch_shapes=[
            pltpu.VMEM((W_SUB, 256, NL), U32),
            pltpu.VMEM((55, 256, NL), U32),
            pltpu.VMEM((55, 256, NL), U32),
            pltpu.VMEM((55, 256, NL), U32),
            pltpu.VMEM((55, 192, NL), U32),
            pltpu.VMEM((55, 64, NL), U32),
            pltpu.VMEM((NSLOT_A, SR, NL), F32),
            pltpu.VMEM((81, 8, M // 2, NL), U32),
            pltpu.VMEM((B, T, D), BF16),
            pltpu.VMEM((B * NU, D), BF16),
            pltpu.VMEM((D, D), BF16),
            pltpu.VMEM((D, D), BF16),
            pltpu.VMEM((D, D), BF16),
            pltpu.VMEM((NCH, 512, NL), BF16),
            pltpu.VMEM((NCH, 512, NL), F32),
            pltpu.VMEM((NCH, 3 * B * NU, NL), F32),
            pltpu.VMEM((8, 512, D), BF16),
            pltpu.SMEM((1,), jnp.int32),
            pltpu.SemaphoreType.DMA((22,)),
            pltpu.SemaphoreType.DMA((11,)),
        ],
        compiler_params=pltpu.CompilerParams(vmem_limit_bytes=120 * 1024 * 1024),
    )(x, w1, w2, g.reshape(B * NU, D), w_f, w_g, w_o)
    return out.reshape(B, 250, NU, D)
```
